```python
import os as _os
_os.environ.setdefault("JAX_PLATFORMS", "cpu")
import jax
import jax.numpy as jnp

def _softmax(x, axis=-1):
    return jax.nn.softmax(x, axis=axis)
def _gelu(x):
    return jax.nn.gelu(x, approximate=True)
def _silu(x):
    return jax.nn.silu(x)
def _sigmoid(x):
    return jax.nn.sigmoid(x)
def _layernorm(x, axis=-1, eps=1e-5):
    m = jnp.mean(x, axis=axis, keepdims=True)
    v = jnp.var(x, axis=axis, keepdims=True)
    return (x - m) / jnp.sqrt(v + eps)
def _scatter_add(tgt, idx, src, axis=0):
    return tgt.at[idx].add(src)
def _segment_sum(src, seg, n):
    return jax.ops.segment_sum(src, seg, n)
class _Rng:
    def __init__(self, key):
        self._k = key
    def _next(self):
        self._k, sub = jax.random.split(self._k)
        return sub
    def normal(self, shape):
        return jax.random.normal(self._next(), shape, dtype=jnp.bfloat16)
    def randint(self, lo, hi, shape):
        return jax.random.randint(self._next(), shape, lo, hi, dtype=jnp.int32)
    def uniform(self, shape, lo=0.0, hi=1.0):
        return jax.random.uniform(self._next(), shape, jnp.bfloat16, lo, hi)
    def permutation(self, n):
        return jax.random.permutation(self._next(), n)


kernel_name = 'gated_mix__ssm_conv_h3__ssm_conv_h3__prompt'

def setup_inputs():
    _rng = _Rng(jax.random.key(int.from_bytes(__import__("os").urandom(4), "little")))
    _w = (lambda a: (lambda t: t.astype(jnp.bfloat16) if jnp.issubdtype(t.dtype, jnp.floating) else t)(jnp.asarray(a)))
    def _A_setup():
        B, S, D = 1, 2048, 640
        ks = 4
        return {
            "q": _w((lambda *s: _rng.normal(s) * 0.05)(B, S, D)),
            "k": _w((lambda *s: _rng.normal(s) * 0.05)(B, S, D)),
            "v": _w((lambda *s: _rng.normal(s) * 0.05)(B, S, D)),
            "shift_k": _w((lambda *s: _rng.normal(s) * 0.05)(D, ks) * 0.5),
            "ssm_k": _w((lambda *s: _rng.normal(s) * 0.05)(D, S) * (1.0 / S ** 0.5)),
            "ssm_D": _w((lambda *s: _rng.normal(s) * 0.05)(D)),
        }
    _A_in = _A_setup()

    def _B_setup():
        B, S, D = 1, 2048, 640
        ks = 4
        return {
            "q": _w((lambda *s: _rng.normal(s) * 0.05)(B, S, D)),
            "k": _w((lambda *s: _rng.normal(s) * 0.05)(B, S, D)),
            "v": _w((lambda *s: _rng.normal(s) * 0.05)(B, S, D)),
            "shift_k": _w((lambda *s: _rng.normal(s) * 0.05)(D, ks) * 0.5),
            "ssm_k": _w((lambda *s: _rng.normal(s) * 0.05)(D, S) * (1.0 / S ** 0.5)),
            "ssm_D": _w((lambda *s: _rng.normal(s) * 0.05)(D)),
        }
    _B_in = _B_setup()

    return {
        "A_q": _A_in["q"],
        "A_k": _A_in["k"],
        "A_v": _A_in["v"],
        "A_shift_k": _A_in["shift_k"],
        "A_ssm_k": _A_in["ssm_k"],
        "A_ssm_D": _A_in["ssm_D"],
        "B_q": _B_in["q"],
        "B_k": _B_in["k"],
        "B_v": _B_in["v"],
        "B_shift_k": _B_in["shift_k"],
        "B_ssm_k": _B_in["ssm_k"],
        "B_ssm_D": _B_in["ssm_D"],
        "gate_w": _w((lambda *s: _rng.normal(s) * 0.05)(640) * 16.0),
    }

def reference(A_q, A_k, A_v, A_shift_k, A_ssm_k, A_ssm_D, B_q, B_k, B_v, B_shift_k, B_ssm_k, B_ssm_D, gate_w):
    def _A_ref(q, k, v, shift_k, ssm_k, ssm_D):
        B, S, D = q.shape
        ks = shift_k.shape[-1]
        k_pad = jnp.pad(k, ((0, 0), (ks - 1, 0), (0, 0)))
        k_shift = jnp.zeros_like(k)
        for t in range(ks):
            k_shift = k_shift + k_pad[:, t:t + S, :] * shift_k[:, ks - 1 - t][None, None, :]
        kv = k_shift * v
        L = 2 * S
        kv_pad = jnp.pad(kv, ((0, 0), (0, S), (0, 0)))
        kf_pad = jnp.pad(ssm_k, ((0, 0), (0, S)))
        kv_f = (lambda x, axes=(-2,-1): jnp.fft.rfft2(x.astype(jnp.float32), axes=axes))(kv_pad[:, None, :, :], axes=(1, 2))
        kf_f = (lambda x, axes=(-2,-1): jnp.fft.rfft2(x.astype(jnp.float32), axes=axes))(kf_pad[:, None, :], axes=(1, 2))
        kf_f = (lambda x, *d: x.transpose(*d))(kf_f, 1, 2, 0)
        y_f = kv_f * kf_f[None, :, :, :]
        y = (lambda x, s, axes=(-2,-1): jnp.fft.irfft2(x, s=s, axes=axes).astype(jnp.bfloat16))(y_f, (1, L), axes=(1, 2))[:, 0, :S, :]
        y = y + kv * ssm_D[None, None, :]
        return q * y

    def _B_ref(q, k, v, shift_k, ssm_k, ssm_D):
        B, S, D = q.shape
        ks = shift_k.shape[-1]
        k_pad = jnp.pad(k, ((0, 0), (ks - 1, 0), (0, 0)))
        k_shift = jnp.zeros_like(k)
        for t in range(ks):
            k_shift = k_shift + k_pad[:, t:t + S, :] * shift_k[:, ks - 1 - t][None, None, :]
        kv = k_shift * v
        L = 2 * S
        kv_pad = jnp.pad(kv, ((0, 0), (0, S), (0, 0)))
        kf_pad = jnp.pad(ssm_k, ((0, 0), (0, S)))
        kv_f = (lambda x, axes=(-2,-1): jnp.fft.rfft2(x.astype(jnp.float32), axes=axes))(kv_pad[:, None, :, :], axes=(1, 2))
        kf_f = (lambda x, axes=(-2,-1): jnp.fft.rfft2(x.astype(jnp.float32), axes=axes))(kf_pad[:, None, :], axes=(1, 2))
        kf_f = (lambda x, *d: x.transpose(*d))(kf_f, 1, 2, 0)
        y_f = kv_f * kf_f[None, :, :, :]
        y = (lambda x, s, axes=(-2,-1): jnp.fft.irfft2(x, s=s, axes=axes).astype(jnp.bfloat16))(y_f, (1, L), axes=(1, 2))[:, 0, :S, :]
        y = y + kv * ssm_D[None, None, :]
        return q * y

    x = A_q
    g = _sigmoid((x * gate_w).sum(-1, keepdims=True))
    a = _A_ref(x, A_k, A_v, A_shift_k, A_ssm_k, A_ssm_D)
    b = _B_ref(x, B_k, B_v, B_shift_k, B_ssm_k, B_ssm_D)
    return g * a + (1 - g) * b
```

```python
import functools
import os

import numpy as np
import jax
import jax.numpy as jnp
from jax import lax
import jax.experimental.pallas as pl
import jax.experimental.pallas.tpu as pltpu


T = 128
N = 2 * T
LW = 128
KS = 4
PAD = 8
RT = int(os.environ.get("K_RT", 16))
PF = int(os.environ.get('K_PF', 3))
GB = int(os.environ.get("K_GB", 4))


def _dft_constants():
    f = np.concatenate([np.arange(0, T, 2), np.arange(1, T, 2)]).astype(np.float64)
    n = np.arange(T, dtype=np.float64)
    theta = np.pi * (2.0 * f[:, None] + 1.0) * n[None, :] / N
    fwd = np.concatenate([np.cos(theta), -np.sin(theta)], axis=0)
    inv = (2.0 / N) * np.concatenate([np.cos(theta).T, -np.sin(theta).T], axis=1)
    return fwd.astype(np.float32), inv.astype(np.float32)


_NT = (((1,), (1,)), ((), ()))


def _kernel(gw_ref, f_in, g_in, ash_ref, bsh_ref, ad_ref, bd_ref,
            q_hbm, ak_hbm, av_hbm, assm_hbm, bk_hbm, bv_hbm, bssm_hbm,
            o_hbm,
            q_buf, k_buf, v_buf, ssm_buf, o_buf,
            f_ref, g_ref, coef_scr, gate_scr, kpad_scr, kv0, kv1, sm0, sm1, u0, u1, h0, h1, y0, y1, yt_scr, yt2_scr, acc_scr,
            in_sem, q_sem, out_sem,
            *, seq, nb, nlg):
    f32 = jnp.float32
    bf16 = jnp.bfloat16
    nsteps = 2 * nlg
    kv_scr, u_scr, h_scr, y_scr = (kv0, kv1), (u0, u1), (h0, h1), (y0, y1)
    sm_scr = (sm0, sm1)
    u32 = jnp.uint32

    def pack(x):
        return pltpu.bitcast(x, u32)

    def unpack(x):
        return pltpu.bitcast(x, bf16)

    nr = T // RT
    bpr = nb // nr

    def in_copies(lg, br):
        s = 2 * lg + br
        k_hbm, v_hbm, ssm_hbm = ((ak_hbm, av_hbm, assm_hbm) if br == 0
                                 else (bk_hbm, bv_hbm, bssm_hbm))
        cols = pl.ds(pl.multiple_of(lg * LW, LW), LW)
        return (
            pltpu.make_async_copy(k_hbm.at[:, cols], k_buf.at[s], in_sem.at[0, s]),
            pltpu.make_async_copy(v_hbm.at[:, cols], v_buf.at[s], in_sem.at[1, s]),
            pltpu.make_async_copy(ssm_hbm.at[cols, :], ssm_buf.at[s], in_sem.at[2, s]),
        )

    def wait_in(s, which):
        if which == 0:
            pltpu.make_async_copy(ak_hbm.at[:, 0:LW], k_buf.at[s], in_sem.at[0, s]).wait()
        elif which == 1:
            pltpu.make_async_copy(av_hbm.at[:, 0:LW], v_buf.at[s], in_sem.at[1, s]).wait()
        else:
            pltpu.make_async_copy(assm_hbm.at[0:LW, :], ssm_buf.at[s], in_sem.at[2, s]).wait()

    q_copy = pltpu.make_async_copy(q_hbm, q_buf, q_sem.at[0])

    def out_copy(lg):
        return pltpu.make_async_copy(
            o_buf.at[lg], o_hbm.at[:, pl.ds(pl.multiple_of(lg * LW, LW), LW)], out_sem.at[lg])

    for s in range(PF):
        for cp in in_copies(s // 2, s % 2):
            cp.start()
        if s == 1:
            q_copy.start()

    eye = (lax.broadcasted_iota(jnp.int32, (8, KS), 0)
           == lax.broadcasted_iota(jnp.int32, (8, KS), 1)).astype(bf16)
    for s in range(nsteps):
        lg, br = s // 2, s % 2
        sh_ref, d_ref = (ash_ref, ad_ref) if br == 0 else (bsh_ref, bd_ref)
        c = lax.dot_general(eye, sh_ref[lg * LW:(lg + 1) * LW, :], _NT,
                            preferred_element_type=f32)
        row = lax.broadcasted_iota(jnp.int32, (8, LW), 0)
        dv = jnp.broadcast_to(d_ref[:, lg * LW:(lg + 1) * LW].astype(f32), (8, LW))
        coef_scr[s] = jnp.where(row == KS, dv, c)
    kpad_scr[0:PAD, :] = jnp.zeros((PAD, LW), f32)
    f_ref[...] = pack(f_in[...])
    g_ref[...] = pack(g_in[...])

    def prep(s, p):
        wait_in(s, 0)
        wait_in(s, 1)
        coef = coef_scr[s]
        kpad_scr[PAD:PAD + seq, :] = k_buf[s].astype(f32)

        def body(j, c):
            r0 = pl.multiple_of(j * T, T)
            ks = kpad_scr[pl.ds(r0 + PAD, T), :] * coef[0:1, :]
            for t in range(1, KS):
                ks = ks + kpad_scr[pl.ds(r0 + (PAD - t), T), :] * coef[t:t + 1, :]
            kv = ks * v_buf[s, pl.ds(r0, T), :].astype(f32)
            kv_scr[p][pl.ds(pl.multiple_of(j * (T // 2), T // 2), T // 2), :] = pack(kv.astype(bf16))
            return c

        lax.fori_loop(0, nb, body, 0)
        wait_in(s, 2)
        sm_scr[p][...] = pack(ssm_buf[s])

    def fwd_u(p, b):
        r0 = pl.multiple_of(b * T, T)
        u_scr[p][:, pl.ds(r0, LW)] = jnp.dot(
            unpack(f_ref[...]),
            unpack(kv_scr[p][pl.ds(pl.multiple_of(b * (T // 2), T // 2), T // 2), :]),
            preferred_element_type=f32)

    def fwd_h(s, p, b):
        r0 = pl.multiple_of(b * T, T)
        h_scr[p][:, pl.ds(r0, LW)] = lax.dot_general(
            unpack(f_ref[...]), unpack(sm_scr[p][:, pl.ds(r0, T)]), _NT,
            preferred_element_type=f32)

    def inv_block(p, b):
        r0 = pl.multiple_of(b * T, T)
        yt_scr[pl.ds(r0, T), :] = jnp.dot(
            unpack(g_ref[:, 0:T]), unpack(y_scr[p][0:T // 2, pl.ds(r0, LW)]),
            preferred_element_type=f32)
        yt2_scr[pl.ds(r0, T), :] = jnp.dot(
            unpack(g_ref[:, T:N]), unpack(y_scr[p][T // 2:T, pl.ds(r0, LW)]),
            preferred_element_type=f32)

    def freq_tile(s, p, r, sign, extra):
        rr = pl.multiple_of(r * RT, RT)
        ri = pl.multiple_of(T + r * RT, RT)
        rr2 = pl.multiple_of(r * (RT // 2), RT // 2)
        ri2 = pl.multiple_of(T // 2 + r * (RT // 2), RT // 2)
        dvec = coef_scr[s][KS:KS + 1, :]
        extra = list(extra)

        def ld(ref, b):
            return (ref[pl.ds(rr, RT), b * LW:(b + 1) * LW],
                    ref[pl.ds(ri, RT), b * LW:(b + 1) * LW])

        prev = None
        for gi in range(nb // GB):
            acc = [None] * GB
            for gj in range(gi + 1):
                if extra:
                    extra.pop(0)()
                us = [ld(u_scr[p], gj * GB + a) for a in range(GB)]
                base = (gi - gj) * GB
                for m in range(max(base - GB + 1, 0), base + GB):
                    hr, hi = ld(h_scr[p], m)
                    if m == 0:
                        hr = hr + dvec
                    for a in range(GB):
                        b = m + a - base
                        if 0 <= b < GB:
                            ur, ui = us[a]
                            pr = ur * hr - ui * hi
                            pi = ur * hi + ui * hr
                            if acc[b] is None:
                                acc[b] = (pr, pi)
                            else:
                                acc[b] = (acc[b][0] + pr, acc[b][1] + pi)
            for b in range(GB):
                i = gi * GB + b
                acc_r, acc_i = acc[b]
                if prev is None:
                    out_r, out_i = acc_r, acc_i
                elif sign > 0:
                    out_r, out_i = acc_r - prev[1], acc_i + prev[0]
                else:
                    out_r, out_i = acc_r + prev[1], acc_i - prev[0]
                y_scr[p][pl.ds(rr2, RT // 2), i * LW:(i + 1) * LW] = pack(out_r.astype(bf16))
                y_scr[p][pl.ds(ri2, RT // 2), i * LW:(i + 1) * LW] = pack(out_i.astype(bf16))
                prev = acc[b]
        for e in extra:
            e()

    def post(lg, p):
        lane0 = pl.multiple_of(lg * LW, LW)

        def body_a(i, c):
            r0 = pl.multiple_of(i * T, T)
            y = yt_scr[pl.ds(r0, T), :] + yt2_scr[pl.ds(r0, T), :]
            acc_scr[pl.ds(r0, T), :] = gate_scr[pl.ds(r0, T), :] * y
            return c

        def body_b(i, c):
            r0 = pl.multiple_of(i * T, T)
            g = gate_scr[pl.ds(r0, T), :]
            y = yt_scr[pl.ds(r0, T), :] + yt2_scr[pl.ds(r0, T), :]
            mix = acc_scr[pl.ds(r0, T), :] + (1.0 - g) * y
            q = q_buf[pl.ds(r0, T), pl.ds(lane0, LW)].astype(f32)
            o_buf[lg, pl.ds(r0, T), :] = (q * mix).astype(bf16)
            return c

        if p == 0:
            lax.fori_loop(0, nb, body_a, 0)
        else:
            lax.fori_loop(0, nb, body_b, 0)
            out_copy(lg).start()

    with jax.named_scope('prologue'):
        prep(0, 0)
        for b in range(nb):
            fwd_u(0, b)
            fwd_h(0, 0, b)
        prep(1, 1)

    def slot(lg, p):
        s = 2 * lg + p
        sn = jnp.minimum(s + 1, nsteps - 1)

        @pl.when(s + PF < nsteps)
        def _():
            for cp in in_copies(lg + (p + PF) // 2, (p + PF) % 2):
                cp.start()

        def tile(r, cc, sign):
            extra = []
            for e in range(bpr):
                b = r * bpr + e
                extra.append(functools.partial(fwd_u, 1 - p, b))
                extra.append(functools.partial(fwd_h, sn, 1 - p, b))
                extra.append(functools.partial(inv_block, 1 - p, b))
            freq_tile(s, p, r, sign, extra)
            return cc

        with jax.named_scope('freq'):
            lax.fori_loop(0, nr // 2, functools.partial(tile, sign=1), 0)
            lax.fori_loop(nr // 2, nr, functools.partial(tile, sign=-1), 0)

        if p == 1:
            @pl.when(lg == 0)
            def _():
                with jax.named_scope('gate'):
                    q_copy.wait()
                    wb = jnp.broadcast_to(gw_ref[...], (LW, gw_ref.shape[1]))
                    z = lax.dot_general(q_buf[...], wb, _NT, preferred_element_type=f32)
                    gate_scr[...] = jax.nn.sigmoid(z)

            with jax.named_scope('post'):
                post(lg, 0)
        else:
            @pl.when(lg >= 1)
            def _():
                with jax.named_scope('post'):
                    post(lg - 1, 1)

        @pl.when(s + 2 < nsteps)
        def _():
            with jax.named_scope('prep'):
                prep(s + 2, p)

    def lane_group(lg, c):
        slot(lg, 0)
        slot(lg, 1)
        return c

    lax.fori_loop(0, nlg, lane_group, 0)

    with jax.named_scope('epilogue'):
        for b in range(nb):
            inv_block(1, b)
        post(nlg - 1, 1)
        for lg in range(nlg):
            out_copy(lg).wait()


@jax.jit
def pallas_gated_mix__ssm_conv_h3__ssm_conv_h3__prompt_kernel(
    A_q: jax.Array,
    A_k: jax.Array,
    A_v: jax.Array,
    A_shift_k: jax.Array,
    A_ssm_k: jax.Array,
    A_ssm_D: jax.Array,
    B_q: jax.Array,
    B_k: jax.Array,
    B_v: jax.Array,
    B_shift_k: jax.Array,
    B_ssm_k: jax.Array,
    B_ssm_D: jax.Array,
    gate_w: jax.Array,
):
    _, S, D = A_q.shape
    nb = S // T
    nlg = D // LW
    nsteps = 2 * nlg
    fwd, inv = _dft_constants()
    fwd = jnp.asarray(fwd, jnp.bfloat16)
    inv = jnp.asarray(inv, jnp.bfloat16)

    vmem = pl.BlockSpec(memory_space=pltpu.VMEM)
    hbm = pl.BlockSpec(memory_space=pl.ANY)
    bf16, f32, u32 = jnp.bfloat16, jnp.float32, jnp.uint32

    out = pl.pallas_call(
        functools.partial(_kernel, seq=S, nb=nb, nlg=nlg),
        in_specs=[vmem] * 7 + [hbm] * 7,
        out_specs=hbm,
        out_shape=jax.ShapeDtypeStruct((S, D), bf16),
        scratch_shapes=[
            pltpu.VMEM((S, D), bf16),
            pltpu.VMEM((nsteps, S, LW), bf16),
            pltpu.VMEM((nsteps, S, LW), bf16),
            pltpu.VMEM((nsteps, LW, S), bf16),
            pltpu.VMEM((nlg, S, LW), bf16),
            pltpu.VMEM((N // 2, T), u32),
            pltpu.VMEM((T // 2, N), u32),
            pltpu.VMEM((nsteps, 8, LW), f32),
            pltpu.VMEM((S, LW), f32),
            pltpu.VMEM((S + PAD, LW), f32),
            pltpu.VMEM((S // 2, LW), u32),
            pltpu.VMEM((S // 2, LW), u32),
            pltpu.VMEM((LW // 2, S), u32),
            pltpu.VMEM((LW // 2, S), u32),
            pltpu.VMEM((N, nb * LW), f32),
            pltpu.VMEM((N, nb * LW), f32),
            pltpu.VMEM((N, nb * LW), f32),
            pltpu.VMEM((N, nb * LW), f32),
            pltpu.VMEM((N // 2, nb * LW), u32),
            pltpu.VMEM((N // 2, nb * LW), u32),
            pltpu.VMEM((S, LW), f32),
            pltpu.VMEM((S, LW), f32),
            pltpu.VMEM((S, LW), f32),
            pltpu.SemaphoreType.DMA((3, nsteps)),
            pltpu.SemaphoreType.DMA((1,)),
            pltpu.SemaphoreType.DMA((nlg,)),
        ],
        compiler_params=pltpu.CompilerParams(
            vmem_limit_bytes=100 * 1024 * 1024,
        ),
    )(
        gate_w.reshape(1, D), fwd, inv, A_shift_k, B_shift_k,
        A_ssm_D.reshape(1, D), B_ssm_D.reshape(1, D),
        A_q.reshape(S, D), A_k.reshape(S, D), A_v.reshape(S, D), A_ssm_k,
        B_k.reshape(S, D), B_v.reshape(S, D), B_ssm_k,
    )
    return out.reshape(1, S, D)
```

```python
import functools
import os

import numpy as np
import jax
import jax.numpy as jnp
from jax import lax
import jax.experimental.pallas as pl
import jax.experimental.pallas.tpu as pltpu


T = 128
N = 2 * T
LW = 128
KS = 4
PAD = 8
RT = int(os.environ.get("K_RT", 16))
PF = int(os.environ.get('K_PF', 4))
NQ = int(os.environ.get('K_NQ', 4))
SB = 16
GB = int(os.environ.get("K_GB", 4))


def _dft_constants():
    f = np.concatenate([np.arange(0, T, 2), np.arange(1, T, 2)]).astype(np.float64)
    n = np.arange(T, dtype=np.float64)
    theta = np.pi * (2.0 * f[:, None] + 1.0) * n[None, :] / N
    fwd = np.concatenate([np.cos(theta), -np.sin(theta)], axis=0)
    inv = (2.0 / N) * np.concatenate([np.cos(theta).T, -np.sin(theta).T], axis=1)
    return fwd.astype(np.float32), inv.astype(np.float32)


_NT = (((1,), (1,)), ((), ()))


def _kernel(gw_ref, f_in, g_in, ash_ref, bsh_ref, ad_ref, bd_ref,
            q_hbm, ak_hbm, av_hbm, assm_hbm, bk_hbm, bv_hbm, bssm_hbm,
            o_hbm,
            q_buf, k_buf, v_buf, ssm_buf, o_buf,
            f_ref, g_ref, coef_scr, gate_scr, kpad_scr, kv0, kv1, sm0, sm1, u0, u1, h0, h1, y0, y1, yta, ytb, yt2a, yt2b,
            in_sem, first_sem, q_sem, out_sem,
            *, seq, nb, nlg):
    f32 = jnp.float32
    bf16 = jnp.bfloat16
    nsteps = 2 * nlg
    kv_scr, u_scr, h_scr, y_scr = (kv0, kv1), (u0, u1), (h0, h1), (y0, y1)
    sm_scr = (sm0, sm1)
    yt_scr, yt2_scr = (yta, ytb), (yt2a, yt2b)
    u32 = jnp.uint32

    def pack(x):
        return pltpu.bitcast(x, u32)

    def unpack(x):
        return pltpu.bitcast(x, bf16)

    nr = T // RT
    bpr = nb // nr

    def in_copies(lg, br):
        s = 2 * lg + br
        k_hbm, v_hbm, ssm_hbm = ((ak_hbm, av_hbm, assm_hbm) if br == 0
                                 else (bk_hbm, bv_hbm, bssm_hbm))
        cols = pl.ds(pl.multiple_of(lg * LW, LW), LW)
        return (
            pltpu.make_async_copy(k_hbm.at[:, cols], k_buf.at[s], in_sem.at[0, s]),
            pltpu.make_async_copy(v_hbm.at[:, cols], v_buf.at[s], in_sem.at[1, s]),
            pltpu.make_async_copy(ssm_hbm.at[cols, :], ssm_buf.at[s], in_sem.at[2, s]),
        )

    def wait_in(s, which):
        if which == 0:
            pltpu.make_async_copy(ak_hbm.at[:, 0:LW], k_buf.at[s], in_sem.at[0, s]).wait()
        elif which == 1:
            pltpu.make_async_copy(av_hbm.at[:, 0:LW], v_buf.at[s], in_sem.at[1, s]).wait()
        else:
            pltpu.make_async_copy(assm_hbm.at[0:LW, :], ssm_buf.at[s], in_sem.at[2, s]).wait()

    q_copy = pltpu.make_async_copy(q_hbm, q_buf, q_sem.at[0])

    def out_copy(lg):
        return pltpu.make_async_copy(
            o_buf.at[lg], o_hbm.at[:, pl.ds(pl.multiple_of(lg * LW, LW), LW)], out_sem.at[lg])

    qr = seq // NQ

    def first_copy(which, c):
        src, dst = (ak_hbm, k_buf) if which == 0 else (av_hbm, v_buf)
        rows = slice(c * qr, (c + 1) * qr)
        return pltpu.make_async_copy(src.at[rows, 0:LW], dst.at[0, rows, :],
                                     first_sem.at[which, c])

    for c in range(NQ):
        first_copy(0, c).start()
        first_copy(1, c).start()
    in_copies(0, 0)[2].start()

    def start_rest():
        for s in range(1, PF):
            for cp in in_copies(s // 2, s % 2):
                cp.start()
            if s == 1:
                q_copy.start()

    for s in range(nsteps):
        lg, br = s // 2, s % 2
        sh_ref, d_ref = (ash_ref, ad_ref) if br == 0 else (bsh_ref, bd_ref)
        cols = slice(lg * LW, (lg + 1) * LW)
        coef_scr[s, 0:KS, :] = sh_ref[:, cols].astype(f32)
        coef_scr[s, KS:KS + 1, :] = d_ref[cols].astype(f32).reshape(1, LW)
    kpad_scr[0:PAD, :] = jnp.zeros((PAD, LW), f32)
    f_ref[...] = pack(f_in[...])
    g_ref[...] = pack(g_in[...])

    def prep(s, p, first=False):
        coef = coef_scr[s, 0:KS, :]

        def body(j, c):
            r0 = pl.multiple_of(j * T, T)
            rn = pl.multiple_of(jnp.minimum(j + 1, nb - 1) * T, T)
            for h in range(T // SB):
                o = h * SB
                ks = kpad_scr[pl.ds(r0 + (PAD + o), SB), :] * coef[0:1, :]
                for t in range(1, KS):
                    ks = ks + kpad_scr[pl.ds(r0 + (PAD + o - t), SB), :] * coef[t:t + 1, :]
                kv = ks * v_buf[s, pl.ds(r0 + o, SB), :].astype(f32)
                kv_scr[p][o // 2:(o + SB) // 2, pl.ds(r0, LW)] = pack(kv.astype(bf16))
            if not first:
                sm_scr[p][:, pl.ds(r0, T)] = pack(ssm_buf[s, :, pl.ds(r0, T)])
            kpad_scr[pl.ds(rn + PAD, T), :] = k_buf[s, pl.ds(rn, T), :].astype(f32)
            return c

        if first:
            bq = nb // NQ
            first_copy(0, 0).wait()
            kpad_scr[PAD:PAD + T, :] = k_buf[s, 0:T, :].astype(f32)
            for c in range(NQ):
                first_copy(1, c).wait()
                if c + 1 < NQ:
                    first_copy(0, c + 1).wait()
                lax.fori_loop(c * bq, (c + 1) * bq, body, 0)
            start_rest()
            wait_in(s, 2)
            sm_scr[p][...] = pack(ssm_buf[s])
        else:
            wait_in(s, 0)
            wait_in(s, 1)
            wait_in(s, 2)
            kpad_scr[PAD:PAD + T, :] = k_buf[s, 0:T, :].astype(f32)
            lax.fori_loop(0, nb, body, 0)

    def fwd_u(p, b):
        r0 = pl.multiple_of(b * T, T)
        u_scr[p][:, pl.ds(r0, LW)] = jnp.dot(
            unpack(f_ref[...]),
            unpack(kv_scr[p][:, pl.ds(r0, LW)]),
            preferred_element_type=f32)

    def fwd_h(s, p, b):
        r0 = pl.multiple_of(b * T, T)
        h_scr[p][:, pl.ds(r0, LW)] = lax.dot_general(
            unpack(f_ref[...]), unpack(sm_scr[p][:, pl.ds(r0, T)]), _NT,
            preferred_element_type=f32)

    def inv_block(p, b):
        r0 = pl.multiple_of(b * T, T)
        yt_scr[p][pl.ds(r0, T), :] = jnp.dot(
            unpack(g_ref[:, 0:T]), unpack(y_scr[p][0:T // 2, pl.ds(r0, LW)]),
            preferred_element_type=f32)
        yt2_scr[p][pl.ds(r0, T), :] = jnp.dot(
            unpack(g_ref[:, T:N]), unpack(y_scr[p][T // 2:T, pl.ds(r0, LW)]),
            preferred_element_type=f32)

    def freq_tile(s, p, r, sign, extra):
        rr = pl.multiple_of(r * RT, RT)
        ri = pl.multiple_of(T + r * RT, RT)
        rr2 = pl.multiple_of(r * (RT // 2), RT // 2)
        ri2 = pl.multiple_of(T // 2 + r * (RT // 2), RT // 2)
        dvec = coef_scr[s, KS:KS + 1, :]
        extra = list(extra)

        def ld(ref, b):
            return (ref[pl.ds(rr, RT), b * LW:(b + 1) * LW],
                    ref[pl.ds(ri, RT), b * LW:(b + 1) * LW])

        prev = None
        for gi in range(nb // GB):
            acc = [None] * GB
            for gj in range(gi + 1):
                if extra:
                    extra.pop(0)()
                us = [ld(u_scr[p], gj * GB + a) for a in range(GB)]
                base = (gi - gj) * GB
                for m in range(max(base - GB + 1, 0), base + GB):
                    hr, hi = ld(h_scr[p], m)
                    if m == 0:
                        hr = hr + dvec
                    for a in range(GB):
                        b = m + a - base
                        if 0 <= b < GB:
                            ur, ui = us[a]
                            pr = ur * hr - ui * hi
                            pi = ur * hi + ui * hr
                            if acc[b] is None:
                                acc[b] = (pr, pi)
                            else:
                                acc[b] = (acc[b][0] + pr, acc[b][1] + pi)
            for b in range(GB):
                i = gi * GB + b
                acc_r, acc_i = acc[b]
                if prev is None:
                    out_r, out_i = acc_r, acc_i
                elif sign > 0:
                    out_r, out_i = acc_r - prev[1], acc_i + prev[0]
                else:
                    out_r, out_i = acc_r + prev[1], acc_i - prev[0]
                y_scr[p][pl.ds(rr2, RT // 2), i * LW:(i + 1) * LW] = pack(out_r.astype(bf16))
                y_scr[p][pl.ds(ri2, RT // 2), i * LW:(i + 1) * LW] = pack(out_i.astype(bf16))
                prev = acc[b]
        for e in extra:
            e()

    def post(lg):
        lane0 = pl.multiple_of(lg * LW, LW)

        def body(i, c):
            r0 = pl.multiple_of(i * T, T)
            rows = pl.ds(r0, T)
            ya = yt_scr[0][rows, :] + yt2_scr[0][rows, :]
            yb = yt_scr[1][rows, :] + yt2_scr[1][rows, :]
            mix = yb + gate_scr[rows, :] * (ya - yb)
            q = q_buf[rows, pl.ds(lane0, LW)].astype(f32)
            o_buf[lg, rows, :] = (q * mix).astype(bf16)
            return c

        lax.fori_loop(0, nb, body, 0)
        out_copy(lg).start()

    with jax.named_scope('prologue'):
        with jax.named_scope('p_prep0'):
            prep(0, 0, first=True)
        with jax.named_scope('p_fwd0'):
            for b in range(nb):
                fwd_u(0, b)
                fwd_h(0, 0, b)
        with jax.named_scope('p_prep1'):
            prep(1, 1)

    def slot(lg, p):
        s = 2 * lg + p
        sn = jnp.minimum(s + 1, nsteps - 1)

        @pl.when(s + PF < nsteps)
        def _():
            for cp in in_copies(lg + (p + PF) // 2, (p + PF) % 2):
                cp.start()

        def tile(r, cc, sign):
            extra = []
            fu = [functools.partial(fwd_u, 1 - p, r * bpr + e) for e in range(bpr)]
            fh = [functools.partial(fwd_h, sn, 1 - p, r * bpr + e) for e in range(bpr)]
            iv = [functools.partial(inv_block, 1 - p, r * bpr + e) for e in range(bpr)]
            ordr = int(os.environ.get('K_ORD', 0))
            if ordr == 0:
                extra = [fu[0], fh[0], iv[0], fu[1], fh[1], iv[1]]
            elif ordr == 1:
                extra = [iv[0], fu[0], fh[0], iv[1], fu[1], fh[1]]
            elif ordr == 2:
                extra = [fu[0], fh[0], fu[1], fh[1], iv[0], iv[1]]
            elif ordr == 3:
                extra = [iv[0], iv[1], fu[0], fh[0], fu[1], fh[1]]
            elif ordr == 4:
                extra = [lambda: [f() for f in (fu[0], fh[0], fu[1], fh[1], iv[0], iv[1])]]
            freq_tile(s, p, r, sign, extra)
            return cc

        with jax.named_scope('freq'):
            lax.fori_loop(0, nr // 2, functools.partial(tile, sign=1), 0)
            lax.fori_loop(nr // 2, nr, functools.partial(tile, sign=-1), 0)

        if p == 1:
            @pl.when(lg == 0)
            def _():
                with jax.named_scope('gate'):
                    q_copy.wait()
                    wb = jnp.broadcast_to(gw_ref[...].reshape(1, -1), (LW, gw_ref.shape[0]))
                    z = lax.dot_general(q_buf[...], wb, _NT, preferred_element_type=f32)
                    gate_scr[...] = jax.nn.sigmoid(z)
        else:
            @pl.when(lg >= 1)
            def _():
                with jax.named_scope('post'):
                    post(lg - 1)

        @pl.when(s + 2 < nsteps)
        def _():
            with jax.named_scope('prep'):
                prep(s + 2, p)

    def lane_group(lg, c):
        slot(lg, 0)
        slot(lg, 1)
        return c

    lax.fori_loop(0, nlg, lane_group, 0)

    with jax.named_scope('epilogue'):
        for b in range(nb):
            inv_block(1, b)
        post(nlg - 1)
        for lg in range(nlg):
            out_copy(lg).wait()


@jax.jit
def pallas_gated_mix__ssm_conv_h3__ssm_conv_h3__prompt_kernel(
    A_q: jax.Array,
    A_k: jax.Array,
    A_v: jax.Array,
    A_shift_k: jax.Array,
    A_ssm_k: jax.Array,
    A_ssm_D: jax.Array,
    B_q: jax.Array,
    B_k: jax.Array,
    B_v: jax.Array,
    B_shift_k: jax.Array,
    B_ssm_k: jax.Array,
    B_ssm_D: jax.Array,
    gate_w: jax.Array,
):
    _, S, D = A_q.shape
    nb = S // T
    nlg = D // LW
    nsteps = 2 * nlg
    fwd, inv = _dft_constants()
    fwd = jnp.asarray(fwd, jnp.bfloat16)
    inv = jnp.asarray(inv, jnp.bfloat16)

    vmem = pl.BlockSpec(memory_space=pltpu.VMEM)
    hbm = pl.BlockSpec(memory_space=pl.ANY)
    bf16, f32, u32 = jnp.bfloat16, jnp.float32, jnp.uint32

    out = pl.pallas_call(
        functools.partial(_kernel, seq=S, nb=nb, nlg=nlg),
        in_specs=[vmem] * 7 + [hbm] * 7,
        out_specs=hbm,
        out_shape=jax.ShapeDtypeStruct((S, D), bf16),
        scratch_shapes=[
            pltpu.VMEM((S, D), bf16),
            pltpu.VMEM((nsteps, S, LW), bf16),
            pltpu.VMEM((nsteps, S, LW), bf16),
            pltpu.VMEM((nsteps, LW, S), bf16),
            pltpu.VMEM((nlg, S, LW), bf16),
            pltpu.VMEM((N // 2, T), u32),
            pltpu.VMEM((T // 2, N), u32),
            pltpu.VMEM((nsteps, 8, LW), f32),
            pltpu.VMEM((S, LW), f32),
            pltpu.VMEM((S + PAD, LW), f32),
            pltpu.VMEM((T // 2, nb * LW), u32),
            pltpu.VMEM((T // 2, nb * LW), u32),
            pltpu.VMEM((LW // 2, S), u32),
            pltpu.VMEM((LW // 2, S), u32),
            pltpu.VMEM((N, nb * LW), f32),
            pltpu.VMEM((N, nb * LW), f32),
            pltpu.VMEM((N, nb * LW), f32),
            pltpu.VMEM((N, nb * LW), f32),
            pltpu.VMEM((N // 2, nb * LW), u32),
            pltpu.VMEM((N // 2, nb * LW), u32),
            pltpu.VMEM((S, LW), f32),
            pltpu.VMEM((S, LW), f32),
            pltpu.VMEM((S, LW), f32),
            pltpu.VMEM((S, LW), f32),
            pltpu.SemaphoreType.DMA((3, nsteps)),
            pltpu.SemaphoreType.DMA((2, NQ)),
            pltpu.SemaphoreType.DMA((1,)),
            pltpu.SemaphoreType.DMA((nlg,)),
        ],
        compiler_params=pltpu.CompilerParams(
            vmem_limit_bytes=100 * 1024 * 1024,
        ),
    )(
        gate_w, fwd, inv, A_shift_k.T, B_shift_k.T, A_ssm_D, B_ssm_D,
        A_q.reshape(S, D), A_k.reshape(S, D), A_v.reshape(S, D), A_ssm_k,
        B_k.reshape(S, D), B_v.reshape(S, D), B_ssm_k,
    )
    return out.reshape(1, S, D)
```

```python
import functools

import numpy as np
import jax
import jax.numpy as jnp
from jax import lax
import jax.experimental.pallas as pl
import jax.experimental.pallas.tpu as pltpu


T = 128
N = 2 * T
LW = 128
KS = 4
PAD = 8
RT = 16
PF = 4
NQ = 4
SB = 16
GB = 4


def _dft_constants():
    f = np.concatenate([np.arange(0, T, 2), np.arange(1, T, 2)]).astype(np.float64)
    n = np.arange(T, dtype=np.float64)
    theta = np.pi * (2.0 * f[:, None] + 1.0) * n[None, :] / N
    fwd = np.concatenate([np.cos(theta), -np.sin(theta)], axis=0)
    inv = (2.0 / N) * np.concatenate([np.cos(theta).T, -np.sin(theta).T], axis=1)
    return fwd.astype(np.float32), inv.astype(np.float32)


_NT = (((1,), (1,)), ((), ()))


def _kernel(gw_ref, f_in, g_in, ash_ref, bsh_ref, ad_ref, bd_ref,
            q_hbm, ak_hbm, av_hbm, assm_hbm, bk_hbm, bv_hbm, bssm_hbm,
            o_hbm,
            q_buf, k_buf, v_buf, ssm_buf, o_buf,
            f_ref, g_ref, coef_scr, gate_scr, kpad_scr,
            kv0, kv1, sm0, sm1, u0, u1, h0, h1, y0, y1, yta, ytb, yt2a, yt2b,
            in_sem, first_sem, q_sem, out_sem,
            *, seq, nb, nlg):
    f32 = jnp.float32
    bf16 = jnp.bfloat16
    nsteps = 2 * nlg
    kv_scr, u_scr, h_scr, y_scr = (kv0, kv1), (u0, u1), (h0, h1), (y0, y1)
    sm_scr = (sm0, sm1)
    yt_scr, yt2_scr = (yta, ytb), (yt2a, yt2b)
    u32 = jnp.uint32

    def pack(x):
        return pltpu.bitcast(x, u32)

    def unpack(x):
        return pltpu.bitcast(x, bf16)

    nr = T // RT
    bpr = nb // nr

    def in_copies(lg, br):
        s = 2 * lg + br
        k_hbm, v_hbm, ssm_hbm = ((ak_hbm, av_hbm, assm_hbm) if br == 0
                                 else (bk_hbm, bv_hbm, bssm_hbm))
        cols = pl.ds(pl.multiple_of(lg * LW, LW), LW)
        return (
            pltpu.make_async_copy(k_hbm.at[:, cols], k_buf.at[s], in_sem.at[0, s]),
            pltpu.make_async_copy(v_hbm.at[:, cols], v_buf.at[s], in_sem.at[1, s]),
            pltpu.make_async_copy(ssm_hbm.at[cols, :], ssm_buf.at[s], in_sem.at[2, s]),
        )

    def wait_in(s, which):
        if which == 0:
            pltpu.make_async_copy(ak_hbm.at[:, 0:LW], k_buf.at[s], in_sem.at[0, s]).wait()
        elif which == 1:
            pltpu.make_async_copy(av_hbm.at[:, 0:LW], v_buf.at[s], in_sem.at[1, s]).wait()
        else:
            pltpu.make_async_copy(assm_hbm.at[0:LW, :], ssm_buf.at[s], in_sem.at[2, s]).wait()

    q_copy = pltpu.make_async_copy(q_hbm, q_buf, q_sem.at[0])

    def out_copy(lg):
        return pltpu.make_async_copy(
            o_buf.at[lg], o_hbm.at[:, pl.ds(pl.multiple_of(lg * LW, LW), LW)], out_sem.at[lg])

    qr = seq // NQ

    def first_copy(which, c):
        src, dst = (ak_hbm, k_buf) if which == 0 else (av_hbm, v_buf)
        rows = slice(c * qr, (c + 1) * qr)
        return pltpu.make_async_copy(src.at[rows, 0:LW], dst.at[0, rows, :],
                                     first_sem.at[which, c])

    for c in range(NQ):
        first_copy(0, c).start()
        first_copy(1, c).start()
    pltpu.make_async_copy(assm_hbm.at[0:LW, :], ssm_buf.at[0], in_sem.at[2, 0]).start()
    for cp in in_copies(0, 1):
        cp.start()

    def start_rest():
        q_copy.start()
        for s in range(2, PF):
            for cp in in_copies(s // 2, s % 2):
                cp.start()

    for s in range(nsteps):
        lg, br = s // 2, s % 2
        sh_ref, d_ref = (ash_ref, ad_ref) if br == 0 else (bsh_ref, bd_ref)
        cols = slice(lg * LW, (lg + 1) * LW)
        coef_scr[s, 0:KS, :] = sh_ref[:, cols].astype(f32)
        coef_scr[s, KS:KS + 1, :] = d_ref[cols].astype(f32).reshape(1, LW)
    kpad_scr[0:PAD, :] = jnp.zeros((PAD, LW), f32)
    f_ref[...] = pack(f_in[...])
    g_ref[...] = pack(g_in[...])

    def prep(s, p, first=False):
        coef = coef_scr[s, 0:KS, :]

        def body(j, c):
            r0 = pl.multiple_of(j * T, T)
            rn = pl.multiple_of(jnp.minimum(j + 1, nb - 1) * T, T)
            for h in range(T // SB):
                o = h * SB
                ks = kpad_scr[pl.ds(r0 + (PAD + o), SB), :] * coef[0:1, :]
                for t in range(1, KS):
                    ks = ks + kpad_scr[pl.ds(r0 + (PAD + o - t), SB), :] * coef[t:t + 1, :]
                kv = ks * v_buf[s, pl.ds(r0 + o, SB), :].astype(f32)
                kv_scr[p][o // 2:(o + SB) // 2, pl.ds(r0, LW)] = pack(kv.astype(bf16))
            if not first:
                sm_scr[p][:, pl.ds(r0, T)] = pack(ssm_buf[s, :, pl.ds(r0, T)])
            kpad_scr[pl.ds(rn + PAD, T), :] = k_buf[s, pl.ds(rn, T), :].astype(f32)
            return c

        if first:
            bq = nb // NQ
            first_copy(0, 0).wait()
            kpad_scr[PAD:PAD + T, :] = k_buf[s, 0:T, :].astype(f32)
            for c in range(NQ):
                first_copy(1, c).wait()
                if c + 1 < NQ:
                    first_copy(0, c + 1).wait()
                lax.fori_loop(c * bq, (c + 1) * bq, body, 0)
            start_rest()
        else:
            wait_in(s, 0)
            wait_in(s, 1)
            wait_in(s, 2)
            kpad_scr[PAD:PAD + T, :] = k_buf[s, 0:T, :].astype(f32)
            lax.fori_loop(0, nb, body, 0)

    def fwd_u(p, b):
        r0 = pl.multiple_of(b * T, T)
        u_scr[p][:, pl.ds(r0, LW)] = jnp.dot(
            unpack(f_ref[...]),
            unpack(kv_scr[p][:, pl.ds(r0, LW)]),
            preferred_element_type=f32)

    def fwd_h(p, b):
        r0 = pl.multiple_of(b * T, T)
        h_scr[p][:, pl.ds(r0, LW)] = lax.dot_general(
            unpack(f_ref[...]), unpack(sm_scr[p][:, pl.ds(r0, T)]), _NT,
            preferred_element_type=f32)

    def inv_block(p, b):
        r0 = pl.multiple_of(b * T, T)
        yt_scr[p][pl.ds(r0, T), :] = jnp.dot(
            unpack(g_ref[:, 0:T]), unpack(y_scr[p][0:T // 2, pl.ds(r0, LW)]),
            preferred_element_type=f32)
        yt2_scr[p][pl.ds(r0, T), :] = jnp.dot(
            unpack(g_ref[:, T:N]), unpack(y_scr[p][T // 2:T, pl.ds(r0, LW)]),
            preferred_element_type=f32)

    def freq_tile(s, p, r, sign, extra):
        rr = pl.multiple_of(r * RT, RT)
        ri = pl.multiple_of(T + r * RT, RT)
        rr2 = pl.multiple_of(r * (RT // 2), RT // 2)
        ri2 = pl.multiple_of(T // 2 + r * (RT // 2), RT // 2)
        dvec = coef_scr[s, KS:KS + 1, :]
        extra = list(extra)

        def ld(ref, b):
            return (ref[pl.ds(rr, RT), b * LW:(b + 1) * LW],
                    ref[pl.ds(ri, RT), b * LW:(b + 1) * LW])

        prev = None
        for gi in range(nb // GB):
            acc = [None] * GB
            for gj in range(gi + 1):
                if extra:
                    extra.pop(0)()
                us = [ld(u_scr[p], gj * GB + a) for a in range(GB)]
                base = (gi - gj) * GB
                for m in range(max(base - GB + 1, 0), base + GB):
                    hr, hi = ld(h_scr[p], m)
                    if m == 0:
                        hr = hr + dvec
                    for a in range(GB):
                        b = m + a - base
                        if 0 <= b < GB:
                            ur, ui = us[a]
                            pr = ur * hr - ui * hi
                            pi = ur * hi + ui * hr
                            if acc[b] is None:
                                acc[b] = (pr, pi)
                            else:
                                acc[b] = (acc[b][0] + pr, acc[b][1] + pi)
            for b in range(GB):
                i = gi * GB + b
                acc_r, acc_i = acc[b]
                if prev is None:
                    out_r, out_i = acc_r, acc_i
                elif sign > 0:
                    out_r, out_i = acc_r - prev[1], acc_i + prev[0]
                else:
                    out_r, out_i = acc_r + prev[1], acc_i - prev[0]
                y_scr[p][pl.ds(rr2, RT // 2), i * LW:(i + 1) * LW] = pack(out_r.astype(bf16))
                y_scr[p][pl.ds(ri2, RT // 2), i * LW:(i + 1) * LW] = pack(out_i.astype(bf16))
                prev = acc[b]
        for e in extra:
            e()

    def post(lg):
        lane0 = pl.multiple_of(lg * LW, LW)

        def body(i, c):
            r0 = pl.multiple_of(i * T, T)
            rows = pl.ds(r0, T)
            ya = yt_scr[0][rows, :] + yt2_scr[0][rows, :]
            yb = yt_scr[1][rows, :] + yt2_scr[1][rows, :]
            mix = yb + gate_scr[rows, :] * (ya - yb)
            q = q_buf[rows, pl.ds(lane0, LW)].astype(f32)
            o_buf[lg, rows, :] = (q * mix).astype(bf16)
            return c

        lax.fori_loop(0, nb, body, 0)
        out_copy(lg).start()

    with jax.named_scope('prologue'):
        with jax.named_scope('p_prep0'):
            prep(0, 0, first=True)
        with jax.named_scope('p_fwd0'):
            for b in range(nb):
                fwd_u(0, b)
            wait_in(0, 2)
            sm_scr[0][...] = pack(ssm_buf[0])
            for b in range(nb):
                fwd_h(0, b)
        with jax.named_scope('p_prep1'):
            prep(1, 1)

    def slot(lg, p):
        s = 2 * lg + p

        @pl.when(s + PF < nsteps)
        def _():
            for cp in in_copies(lg + (p + PF) // 2, (p + PF) % 2):
                cp.start()

        def tile(r, cc, sign):
            extra = []
            for e in range(bpr):
                b = r * bpr + e
                extra.append(functools.partial(fwd_u, 1 - p, b))
                extra.append(functools.partial(fwd_h, 1 - p, b))
                extra.append(functools.partial(inv_block, 1 - p, b))
            freq_tile(s, p, r, sign, extra)
            return cc

        with jax.named_scope('freq'):
            lax.fori_loop(0, nr // 2, functools.partial(tile, sign=1), 0)
            lax.fori_loop(nr // 2, nr, functools.partial(tile, sign=-1), 0)

        if p == 1:
            @pl.when(lg == 0)
            def _():
                with jax.named_scope('gate'):
                    q_copy.wait()
                    wb = jnp.broadcast_to(gw_ref[...].reshape(1, -1), (LW, gw_ref.shape[0]))
                    z = lax.dot_general(q_buf[...], wb, _NT, preferred_element_type=f32)
                    gate_scr[...] = jax.nn.sigmoid(z)
        else:
            @pl.when(lg >= 1)
            def _():
                with jax.named_scope('post'):
                    post(lg - 1)

        @pl.when(s + 2 < nsteps)
        def _():
            with jax.named_scope('prep'):
                prep(s + 2, p)

    def lane_group(lg, c):
        slot(lg, 0)
        slot(lg, 1)
        return c

    lax.fori_loop(0, nlg, lane_group, 0)

    with jax.named_scope('epilogue'):
        for b in range(nb):
            inv_block(1, b)
        post(nlg - 1)
        for lg in range(nlg):
            out_copy(lg).wait()


@jax.jit
def pallas_gated_mix__ssm_conv_h3__ssm_conv_h3__prompt_kernel(
    A_q: jax.Array,
    A_k: jax.Array,
    A_v: jax.Array,
    A_shift_k: jax.Array,
    A_ssm_k: jax.Array,
    A_ssm_D: jax.Array,
    B_q: jax.Array,
    B_k: jax.Array,
    B_v: jax.Array,
    B_shift_k: jax.Array,
    B_ssm_k: jax.Array,
    B_ssm_D: jax.Array,
    gate_w: jax.Array,
):
    _, S, D = A_q.shape
    nb = S // T
    nlg = D // LW
    nsteps = 2 * nlg
    fwd, inv = _dft_constants()
    fwd = jnp.asarray(fwd, jnp.bfloat16)
    inv = jnp.asarray(inv, jnp.bfloat16)

    vmem = pl.BlockSpec(memory_space=pltpu.VMEM)
    hbm = pl.BlockSpec(memory_space=pl.ANY)
    bf16, f32, u32 = jnp.bfloat16, jnp.float32, jnp.uint32

    out = pl.pallas_call(
        functools.partial(_kernel, seq=S, nb=nb, nlg=nlg),
        in_specs=[vmem] * 7 + [hbm] * 7,
        out_specs=hbm,
        out_shape=jax.ShapeDtypeStruct((S, D), bf16),
        scratch_shapes=[
            pltpu.VMEM((S, D), bf16),
            pltpu.VMEM((nsteps, S, LW), bf16),
            pltpu.VMEM((nsteps, S, LW), bf16),
            pltpu.VMEM((nsteps, LW, S), bf16),
            pltpu.VMEM((nlg, S, LW), bf16),
            pltpu.VMEM((N // 2, T), u32),
            pltpu.VMEM((T // 2, N), u32),
            pltpu.VMEM((nsteps, 8, LW), f32),
            pltpu.VMEM((S, LW), f32),
            pltpu.VMEM((S + PAD, LW), f32),
            pltpu.VMEM((T // 2, nb * LW), u32),
            pltpu.VMEM((T // 2, nb * LW), u32),
            pltpu.VMEM((LW // 2, S), u32),
            pltpu.VMEM((LW // 2, S), u32),
            pltpu.VMEM((N, nb * LW), f32),
            pltpu.VMEM((N, nb * LW), f32),
            pltpu.VMEM((N, nb * LW), f32),
            pltpu.VMEM((N, nb * LW), f32),
            pltpu.VMEM((N // 2, nb * LW), u32),
            pltpu.VMEM((N // 2, nb * LW), u32),
            pltpu.VMEM((S, LW), f32),
            pltpu.VMEM((S, LW), f32),
            pltpu.VMEM((S, LW), f32),
            pltpu.VMEM((S, LW), f32),
            pltpu.SemaphoreType.DMA((3, nsteps)),
            pltpu.SemaphoreType.DMA((2, NQ)),
            pltpu.SemaphoreType.DMA((1,)),
            pltpu.SemaphoreType.DMA((nlg,)),
        ],
        compiler_params=pltpu.CompilerParams(
            vmem_limit_bytes=100 * 1024 * 1024,
        ),
    )(
        gate_w, fwd, inv, A_shift_k.T, B_shift_k.T, A_ssm_D, B_ssm_D,
        A_q.reshape(S, D), A_k.reshape(S, D), A_v.reshape(S, D), A_ssm_k,
        B_k.reshape(S, D), B_v.reshape(S, D), B_ssm_k,
    )
    return out.reshape(1, S, D)
```
